```python
import os as _os
_os.environ.setdefault("JAX_PLATFORMS", "cpu")
import jax
import jax.numpy as jnp

def _softmax(x, axis=-1):
    return jax.nn.softmax(x, axis=axis)
def _gelu(x):
    return jax.nn.gelu(x, approximate=True)
def _silu(x):
    return jax.nn.silu(x)
def _sigmoid(x):
    return jax.nn.sigmoid(x)
def _layernorm(x, axis=-1, eps=1e-5):
    m = jnp.mean(x, axis=axis, keepdims=True)
    v = jnp.var(x, axis=axis, keepdims=True)
    return (x - m) / jnp.sqrt(v + eps)
def _scatter_add(tgt, idx, src, axis=0):
    return tgt.at[idx].add(src)
def _segment_sum(src, seg, n):
    return jax.ops.segment_sum(src, seg, n)
class _Rng:
    def __init__(self, key):
        self._k = key
    def _next(self):
        self._k, sub = jax.random.split(self._k)
        return sub
    def normal(self, shape):
        return jax.random.normal(self._next(), shape, dtype=jnp.bfloat16)
    def randint(self, lo, hi, shape):
        return jax.random.randint(self._next(), shape, lo, hi, dtype=jnp.int32)
    def uniform(self, shape, lo=0.0, hi=1.0):
        return jax.random.uniform(self._next(), shape, jnp.bfloat16, lo, hi)
    def permutation(self, n):
        return jax.random.permutation(self._next(), n)


kernel_name = 'concat_heads__grouped_kv_mqa__sliding_block__prompt'

def setup_inputs():
    _rng = _Rng(jax.random.key(int.from_bytes(__import__("os").urandom(4), "little")))
    _w = (lambda a: (lambda t: t.astype(jnp.bfloat16) if jnp.issubdtype(t.dtype, jnp.floating) else t)(jnp.asarray(a)))
    def _A_setup():
        B, S, D, H = 1, 2048, 1024, 32
        Dh = D // H
        return {
            "x": _w((lambda *s: _rng.normal(s) * 0.05)(B, S, D)),
            "wq": _w((lambda *s: _rng.normal(s) * 1.6)(D, H * Dh)),
            "wk": _w((lambda *s: _rng.normal(s) * 1.6)(D, Dh)),
            "wv": _w((lambda *s: _rng.normal(s) * 0.1)(D, Dh)),
            "wo": _w((lambda *s: _rng.normal(s) * 0.1)(H * Dh, D)),
        }
    _A_in = _A_setup()

    def _B_setup():
        B, S, D = 1, 2048, 1024
        return {
            "x": _w((lambda *s: _rng.normal(s) * 0.2)(B, S, D)),
            "wqkv": _w((lambda *s: _rng.normal(s) * 0.2)(D, 3 * D)),
            "wo": _w((lambda *s: _rng.normal(s) * 0.05)(D, D)),
        }
    _B_in = _B_setup()

    return {
        "A_x": _A_in["x"],
        "A_wq": _A_in["wq"],
        "A_wk": _A_in["wk"],
        "A_wv": _A_in["wv"],
        "A_wo": _A_in["wo"],
        "B_x": _B_in["x"],
        "B_wqkv": _B_in["wqkv"],
        "B_wo": _B_in["wo"],
    }

def reference(A_x, A_wq, A_wk, A_wv, A_wo, B_x, B_wqkv, B_wo):
    def _A_ref(x, wq, wk, wv, wo):
        B, S, D = x.shape
        H = 32
        Dh = D // H
        q = (lambda x, *d: x.transpose(*d))((x @ wq).reshape(B, S, H, Dh), 0, 2, 1, 3)
        k = x @ wk
        v = x @ wv
        scores = jnp.einsum("bhqd,bkd->bhqk", q, k) * (Dh ** -0.5)
        p = _softmax(scores, axis=-1)
        o = jnp.einsum("bhqk,bkd->bhqd", p, v)
        return (lambda x, *d: x.transpose(*d))(o, 0, 2, 1, 3).reshape(B, S, H * Dh) @ wo

    def _B_ref(x, wqkv, wo):
        B, S, D = x.shape
        H = 32; Dh = D // H; W = 256
        qkv = (lambda x, *d: x.transpose(*d))((x @ wqkv).reshape(B, S, 3, H, Dh), 2, 0, 3, 1, 4)
        q, k, v = qkv[0], qkv[1], qkv[2]
        scores = jnp.einsum("bhqd,bhkd->bhqk", q, k) * (Dh ** -0.5)
        idx = jnp.arange(S)
        mask = (idx[:, None] - idx[None, :] >= 0) & (idx[:, None] - idx[None, :] < W)
        scores = jnp.where(mask[None, None], scores, -1e9)
        p = _softmax(scores, axis=-1)
        o = jnp.einsum("bhqk,bhkd->bhqd", p, v)
        return (lambda x, *d: x.transpose(*d))(o, 0, 2, 1, 3).reshape(B, S, D) @ wo

    a = _A_ref(A_x, A_wq, A_wk, A_wv, A_wo)
    b = _B_ref(B_x, B_wqkv, B_wo)
    return jnp.concatenate([a, b], axis=-1)
```

```python
import functools

import jax
import jax.numpy as jnp
import jax.experimental.pallas as pl
import jax.experimental.pallas.tpu as pltpu

S = 2048
D = 1024
DH = 32
W = 256
TQ = 128
NT = S // TQ
NG = D // 128
LOG2E = 1.4426950408889634
QSCALE = float(DH ** -0.5) * LOG2E
NEG = -1e9 * LOG2E

KCA = 128
KB = W + TQ
RC = 512

F32 = jnp.float32
BF16 = jnp.bfloat16

_TN_NT = (((0,), (1,)), ((), ()))
_TN = (((0,), (0,)), ((), ()))


def _colmax(s):
    return jnp.max(s.reshape(s.shape[0] // 8, 8, s.shape[1]), axis=0)


def _finmax(m):
    return jnp.broadcast_to(jnp.max(m, axis=0, keepdims=True), m.shape)


def _kernel(xa_hbm, wq_hbm, wk_hbm, wv_hbm, woa_hbm, xb_hbm, wqkv_hbm, wob_hbm,
            out_hbm,
            xa, wq, wk, wv, woa, xb, wqkv, wob,
            qt, ka, vta, ot, s0, s1, m_ref, kb, vtb, bias, obuf,
            in_sems, out_sems):
    cp_wk = pltpu.make_async_copy(wk_hbm, wk, in_sems.at[0])
    cp_wv = pltpu.make_async_copy(wv_hbm, wv, in_sems.at[1])
    cp_xa = pltpu.make_async_copy(xa_hbm, xa, in_sems.at[2])
    cp_wq = pltpu.make_async_copy(wq_hbm, wq, in_sems.at[3])
    cp_woa = pltpu.make_async_copy(woa_hbm, woa, in_sems.at[4])
    cp_xb = pltpu.make_async_copy(xb_hbm, xb, in_sems.at[5])
    cp_wqkv = pltpu.make_async_copy(wqkv_hbm, wqkv, in_sems.at[6])
    cp_wob = pltpu.make_async_copy(wob_hbm, wob, in_sems.at[7])
    for cp in (cp_wk, cp_wv, cp_xa, cp_wq):
        cp.start()

    def out_copy(slot, row, col):
        return pltpu.make_async_copy(
            obuf.at[slot], out_hbm.at[pl.ds(row, RC), pl.ds(col, D)], out_sems.at[slot])

    def out_proj(wo, col):
        for j in range(S // RC):
            slot = j % 2
            o_t = jnp.concatenate([ot[4 * j + i] for i in range(RC // TQ)], axis=1)
            r = jax.lax.dot_general(o_t, wo[...], _TN, preferred_element_type=F32)
            if j >= 2 or col > 0:
                out_copy(slot, 0, 0).wait()
            obuf[slot] = r.astype(BF16)
            out_copy(slot, j * RC, col).start()

    def proj_t(w, x, dst, off, scale=None):
        def body(j, c):
            r0 = pl.multiple_of(j * RC, RC)
            r = jax.lax.dot_general(w[...], x[pl.ds(r0, RC), :], _TN_NT,
                                    preferred_element_type=F32)
            if scale is not None:
                r = r * scale
            r = r.astype(BF16)
            for i in range(RC // TQ):
                dst[off + 4 * j + i] = r[:, i * TQ:(i + 1) * TQ]
            return c
        jax.lax.fori_loop(0, S // RC, body, 0)

    cp_wk.wait()
    cp_wv.wait()
    cp_xa.wait()

    def kv_body(j, c):
        r0 = pl.multiple_of(j * RC, RC)
        x = xa[pl.ds(r0, RC), :]
        ka[pl.ds(r0, RC), :] = jnp.dot(x, wk[...], preferred_element_type=F32).astype(BF16)
        v_t = jax.lax.dot_general(wv[...], x, _TN_NT, preferred_element_type=F32)
        vta[j] = v_t.astype(BF16)
        return c
    jax.lax.fori_loop(0, S // RC, kv_body, 0)

    cp_wq.wait()
    for cp in (cp_woa, cp_xb, cp_wqkv, cp_wob):
        cp.start()
    proj_t(wq, xa, qt, 0, QSCALE)

    sbuf = (s0, s1)
    nca = S // KCA

    def a_load_q(u):
        t = u // NG
        g = u % NG
        q = qt[t, pl.ds(pl.multiple_of(g * 128, 128), 128), :]
        return jnp.concatenate([q[DH * j:DH * (j + 1), :] for j in range(4)], axis=1)

    def a_qk(q, kc, s_ref, m):
        s = jnp.dot(ka[kc * KCA:(kc + 1) * KCA, :], q, preferred_element_type=F32)
        s_ref[kc * KCA:(kc + 1) * KCA, :] = s
        mc = _colmax(s)
        return mc if m is None else jnp.maximum(m, mc)

    def a_step(u, par, do_next=True):
        s_cur, s_nxt = sbuf[par], sbuf[1 - par]
        m_cur = m_ref[par, 0]
        m_nxt = l = o = None
        if do_next:
            q = a_load_q(u + 1)
        for kc in range(nca):
            if do_next:
                m_nxt = a_qk(q, kc, s_nxt, m_nxt)
            s = s_cur[kc * KCA:(kc + 1) * KCA, :].reshape(KCA // 8, 8, 512)
            p = jnp.exp2(s - m_cur[None])
            lc = jnp.sum(p, axis=0)
            l = lc if l is None else l + lc
            v_t = vta[(kc * KCA) // RC, :, (kc * KCA) % RC:(kc * KCA) % RC + KCA]
            oc = jnp.dot(v_t, p.reshape(KCA, 512).astype(BF16), preferred_element_type=F32)
            o = oc if o is None else o + oc
        l = jnp.sum(l, axis=0, keepdims=True)
        o = (o * (1.0 / l)).astype(BF16)
        o = jnp.concatenate([o[:, j * TQ:(j + 1) * TQ] for j in range(4)], axis=0)
        ot[u // NG, pl.ds(pl.multiple_of((u % NG) * 128, 128), 128), :] = o
        if do_next:
            m_ref[1 - par, 0] = _finmax(m_nxt)

    q = a_load_q(0)
    m = None
    for kc in range(nca):
        m = a_qk(q, kc, s0, m)
    m_ref[0, 0] = _finmax(m)

    nua = NT * NG

    def a_body(u, c):
        @pl.when(u % 2 == 0)
        def _():
            a_step(u, 0)

        @pl.when(u % 2 == 1)
        def _():
            a_step(u, 1)
        return c
    jax.lax.fori_loop(0, nua - 1, a_body, 0)
    a_step(nua - 1, (nua - 1) % 2, do_next=False)

    cp_woa.wait()
    out_proj(woa, 0)

    r = jax.lax.broadcasted_iota(jnp.int32, (KB, TQ), 0)
    i = jax.lax.broadcasted_iota(jnp.int32, (KB, TQ), 1)
    band = (r > i) & (r <= i + W)
    for v in range(3):
        bias[v] = jnp.where(band & (r >= W - TQ * v), 0.0, NEG).astype(F32)
    for g in range(NG):
        kb[g, 0:W, :] = jnp.zeros((W, 128), BF16)
    for t in range(W // TQ):
        vtb[t] = jnp.zeros((D, TQ), BF16)

    cp_xb.wait()
    cp_wqkv.wait()

    def kb_body(j, c):
        r0 = pl.multiple_of(j * RC, RC)
        k = jnp.dot(xb[pl.ds(r0, RC), :], wqkv[:, D:2 * D], preferred_element_type=F32).astype(BF16)
        for g in range(NG):
            kb[g, pl.ds(r0 + W, RC), :] = k[:, g * 128:(g + 1) * 128]
        return c
    jax.lax.fori_loop(0, S // RC, kb_body, 0)
    proj_t(wqkv.at[:, 0:D], xb, qt, 0, QSCALE)
    proj_t(wqkv.at[:, 2 * D:3 * D], xb, vtb, W // TQ)

    def b_qk(t, g, s_ref):
        q = qt[t, g * 128:(g + 1) * 128, :]
        z = jnp.zeros((DH, TQ), BF16)
        qm = jnp.concatenate(
            [jnp.concatenate([q[DH * jj:DH * (jj + 1), :] if jj == j else z for jj in range(4)], axis=0)
             for j in range(4)], axis=1)
        k = kb[g, pl.ds(pl.multiple_of(t * TQ, TQ), KB), :]
        s = jnp.dot(k, qm, preferred_element_type=F32)
        b = bias[jnp.minimum(t, 2)]
        s = s + jnp.concatenate([b] * 4, axis=1)
        s_ref[g * KB:(g + 1) * KB, :] = s
        return _finmax(_colmax(s))

    def b_step(t, par, do_next=True):
        s_cur, s_nxt = sbuf[par], sbuf[1 - par]
        for g in range(NG):
            if do_next:
                m_ref[1 - par, g] = b_qk(t + 1, g, s_nxt)
            s = s_cur[g * KB:(g + 1) * KB, :].reshape(KB // 8, 8, 512)
            p = jnp.exp2(s - m_ref[par, g][None])
            l = jnp.sum(jnp.sum(p, axis=0), axis=0, keepdims=True)
            p = p.reshape(KB, 512).astype(BF16)
            inv = 1.0 / l
            os_ = []
            for j in range(4):
                rows = slice(g * 128 + DH * j, g * 128 + DH * (j + 1))
                v_t = jnp.concatenate([vtb[t + a, rows, :] for a in range(KB // TQ)], axis=1)
                o = jnp.dot(v_t, p[:, j * TQ:(j + 1) * TQ], preferred_element_type=F32)
                os_.append((o * inv[:, j * TQ:(j + 1) * TQ]).astype(BF16))
            ot[t, g * 128:(g + 1) * 128, :] = jnp.concatenate(os_, axis=0)

    for g in range(NG):
        m_ref[0, g] = b_qk(0, g, s0)

    def b_body(t, c):
        @pl.when(t % 2 == 0)
        def _():
            b_step(t, 0)

        @pl.when(t % 2 == 1)
        def _():
            b_step(t, 1)
        return c
    jax.lax.fori_loop(0, NT - 1, b_body, 0)
    b_step(NT - 1, (NT - 1) % 2, do_next=False)

    cp_wob.wait()
    out_proj(wob, D)
    out_copy(0, 0, 0).wait()
    out_copy(1, 0, 0).wait()


@jax.jit
def pallas_concat_heads__grouped_kv_mqa__sliding_block__prompt_kernel(
    A_x: jax.Array,
    A_wq: jax.Array,
    A_wk: jax.Array,
    A_wv: jax.Array,
    A_wo: jax.Array,
    B_x: jax.Array,
    B_wqkv: jax.Array,
    B_wo: jax.Array,
):
    hbm = pl.BlockSpec(memory_space=pl.ANY)
    scratch = [
        pltpu.VMEM((S, D), BF16),
        pltpu.VMEM((D, D), BF16),
        pltpu.VMEM((D, DH), BF16),
        pltpu.VMEM((D, DH), BF16),
        pltpu.VMEM((D, D), BF16),
        pltpu.VMEM((S, D), BF16),
        pltpu.VMEM((D, 3 * D), BF16),
        pltpu.VMEM((D, D), BF16),
        pltpu.VMEM((NT, D, TQ), BF16),
        pltpu.VMEM((S, DH), BF16),
        pltpu.VMEM((S // RC, DH, RC), BF16),
        pltpu.VMEM((NT, D, TQ), BF16),
        pltpu.VMEM((NG * KB, 512), F32),
        pltpu.VMEM((NG * KB, 512), F32),
        pltpu.VMEM((2, NG, 8, 512), F32),
        pltpu.VMEM((NG, S + W, 128), BF16),
        pltpu.VMEM((NT + W // TQ, D, TQ), BF16),
        pltpu.VMEM((3, KB, TQ), F32),
        pltpu.VMEM((2, RC, D), BF16),
        pltpu.SemaphoreType.DMA((8,)),
        pltpu.SemaphoreType.DMA((2,)),
    ]
    out = pl.pallas_call(
        _kernel,
        out_shape=jax.ShapeDtypeStruct((S, 2 * D), BF16),
        in_specs=[hbm] * 8,
        out_specs=hbm,
        scratch_shapes=scratch,
        compiler_params=pltpu.CompilerParams(vmem_limit_bytes=100 * 2**20),
    )(A_x.reshape(S, D), A_wq, A_wk, A_wv, A_wo, B_x.reshape(S, D), B_wqkv, B_wo)
    return out.reshape(1, S, 2 * D)
```

```python
import functools

import jax
import jax.numpy as jnp
import jax.experimental.pallas as pl
import jax.experimental.pallas.tpu as pltpu

S = 2048
D = 1024
DH = 32
W = 256
TQ = 128
NT = S // TQ
NG = D // 128
LOG2E = 1.4426950408889634
QSCALE = float(DH ** -0.5) * LOG2E
NEG = -1e9 * LOG2E

KCA = 128
KB = W + TQ
RC = 512
GA = 4
TB = 2
NX0 = 4
NWQ = 4
NLAST = 4
LDEP = True
LDEPB = 2
SROWS = max(GA * S, TB * NG * KB)

F32 = jnp.float32
BF16 = jnp.bfloat16

_TN_NT = (((0,), (1,)), ((), ()))
_TN = (((0,), (0,)), ((), ()))
_NT = (((1,), (1,)), ((), ()))


def _colmax(s):
    return jnp.max(s.reshape(s.shape[0] // 8, 8, s.shape[1]), axis=0)


def _after(x, dep):
    zero = jax.lax.shift_right_logical(
        jax.lax.shift_right_logical(pltpu.bitcast(dep, jnp.uint32), jnp.uint32(31)), jnp.uint32(1))
    return pltpu.bitcast(pltpu.bitcast(x, jnp.uint32) | zero, x.dtype)


def _finmax(m):
    return jnp.broadcast_to(jnp.max(m, axis=0, keepdims=True), m.shape)


def _kernel(xa_hbm, wq_hbm, wk_hbm, wv_hbm, woa_hbm, xb_hbm, wqkv_hbm, wob_hbm,
            out_hbm,
            xa, wq, wkv, woa, xb, wqkv, wob,
            qt, ka, vta, ot, s0, s1, m_ref, kb, vtb, bias,
            sem_wkv, sem_wq, sem_x0, sem_xa, sem_b, sem_out, sem_last):
    nrc = S // RC
    KQ = D // NWQ

    def rows(hbm, vm, r0, n, sem):
        return pltpu.make_async_copy(hbm.at[pl.ds(r0, n)], vm.at[pl.ds(r0, n)], sem)

    cp_wk = pltpu.make_async_copy(wk_hbm, wkv.at[0:DH], sem_wkv.at[0])
    cp_wv = pltpu.make_async_copy(wv_hbm, wkv.at[DH:2 * DH], sem_wkv.at[1])
    cp_wq = [rows(wq_hbm, wq, i * KQ, KQ, sem_wq.at[i]) for i in range(NWQ)]
    cp_x0 = [rows(xa_hbm, xa, i * (RC // NX0), RC // NX0, sem_x0.at[i]) for i in range(NX0)]
    cp_xa = [rows(xa_hbm, xa, j * RC, RC, sem_xa.at[j]) for j in range(1, nrc)]
    cp_woa = pltpu.make_async_copy(woa_hbm, woa, sem_b.at[0])
    cp_xb = pltpu.make_async_copy(xb_hbm, xb, sem_b.at[1])
    cp_wqkv = pltpu.make_async_copy(wqkv_hbm, wqkv, sem_b.at[2])
    cp_wob = pltpu.make_async_copy(wob_hbm, wob, sem_b.at[3])
    for cp in (cp_wk, cp_wv, *cp_x0, cp_wq[0]):
        cp.start()

    def out_copy(buf, col, j):
        return pltpu.make_async_copy(
            buf.at[pl.ds(j * RC, RC)], out_hbm.at[pl.ds(j * RC, RC), pl.ds(col, D)],
            sem_out.at[col // D, j])

    def o_chunk_t(j):
        return jnp.concatenate([ot[(RC // TQ) * j + i] for i in range(RC // TQ)], axis=1)

    def out_proj(wo, buf, col, first):
        prev = None
        for j in range(first, nrc):
            r = jax.lax.dot_general(o_chunk_t(j), wo[...], _TN, preferred_element_type=F32)
            if prev is not None:
                buf[(j - 1) * RC:j * RC, :] = prev
                out_copy(buf, col, j - 1).start()
            prev = r.astype(BF16)
        buf[(nrc - 1) * RC:nrc * RC, :] = prev
        out_copy(buf, col, nrc - 1).start()

    def store_t(r, j, dst, off):
        for i in range(RC // TQ):
            dst[off + (RC // TQ) * j + i] = r[:, i * TQ:(i + 1) * TQ]

    def proj_t(w, x, scale=None):
        r = jax.lax.dot_general(w, x, _TN_NT, preferred_element_type=F32)
        if scale is not None:
            r = r * scale
        return r.astype(BF16)

    r = jax.lax.broadcasted_iota(jnp.int32, (TQ, TQ), 0)
    i = jax.lax.broadcasted_iota(jnp.int32, (TQ, TQ), 1)
    bias[0] = jnp.where(r > i, 0.0, NEG).astype(F32)
    bias[1] = jnp.where(r <= i, 0.0, NEG).astype(F32)

    def a_kv(j):
        kv_t = jax.lax.dot_general(wkv[...], xa[j * RC:(j + 1) * RC, :], _NT,
                                   preferred_element_type=F32)
        ka[j * RC:(j + 1) * RC, :] = kv_t[0:DH].T.astype(BF16)
        vta[j] = kv_t[DH:2 * DH].astype(BF16)

    cp_wk.wait()
    cp_wv.wait()
    for cp in cp_x0:
        cp.wait()
    later = [*cp_wq[1:], *cp_xa]
    later.pop(0).start()
    a_kv(0)
    r = None
    for i in range(NWQ):
        cp_wq[i].wait()
        if later:
            later.pop(0).start()
        ri = jnp.dot(xa[0:RC, i * KQ:(i + 1) * KQ], wq[i * KQ:(i + 1) * KQ, :],
                     preferred_element_type=F32)
        r = ri if r is None else r + ri
    prev = (r * QSCALE).astype(BF16).T
    while later:
        later.pop(0).start()
    for j in range(1, nrc):
        cp_xa[j - 1].wait()
        a_kv(j)
        r = proj_t(wq[...], xa[j * RC:(j + 1) * RC, :], QSCALE)
        store_t(prev, j - 1, qt, 0)
        prev = r
    store_t(prev, nrc - 1, qt, 0)
    for cp in (cp_woa, cp_xb, cp_wqkv, cp_wob):
        cp.start()

    sbuf = (s0, s1)
    nca = S // KCA

    def normalise(o, l):
        r = pl.reciprocal(l, approx=True)
        return o * (r * (2.0 - l * r))

    def a_load_q(t, g):
        q = qt[t, g * 128:(g + 1) * 128, :]
        return jnp.concatenate([q[DH * j:DH * (j + 1), :] for j in range(4)], axis=1)

    def a_qk(q, kc, s_ref, row0, m):
        s = jnp.dot(ka[kc * KCA:(kc + 1) * KCA, :], q, preferred_element_type=F32)
        s_ref[row0 + kc * KCA:row0 + (kc + 1) * KCA, :] = s
        mc = _colmax(s)
        return mc if m is None else jnp.maximum(m, mc)

    def a_step(t, par, do_next=True, filler=None):
        s_cur, s_nxt = sbuf[par], sbuf[1 - par]
        for gi in range(GA):
            g = GA * par + gi
            row0 = gi * S
            m_cur = m_ref[par, gi]
            m_nxt = l = l_old = o = None
            if do_next:
                q = a_load_q(t + par, GA * (1 - par) + gi)
            for kc in range(nca):
                if do_next:
                    m_nxt = a_qk(q, kc, s_nxt, row0, m_nxt)
                if filler is not None:
                    filler(gi * nca + kc)
                s = s_cur[row0 + kc * KCA:row0 + (kc + 1) * KCA, :].reshape(KCA // 8, 8, 512)
                mm = m_cur if (l_old is None or not LDEP) else _after(m_cur, l_old)
                p = jnp.exp2(s - mm[None])
                lc = jnp.sum(p, axis=0)
                l_old, l = l, (lc if l is None else l + lc)
                k0 = kc * KCA
                v_t = vta[k0 // RC, :, k0 % RC:k0 % RC + KCA]
                oc = jnp.dot(v_t, p.reshape(KCA, 512).astype(BF16), preferred_element_type=F32)
                o = oc if o is None else o + oc
            o = normalise(o, jnp.sum(l, axis=0, keepdims=True))
            ot[t, g * 128:(g + 1) * 128, :] = jnp.concatenate(
                [o[:, j * TQ:(j + 1) * TQ].astype(BF16) for j in range(4)], axis=0)
            if do_next:
                m_ref[1 - par, gi] = _finmax(m_nxt)

    for gi in range(GA):
        q = a_load_q(0, gi)
        m = None
        for kc in range(nca):
            m = a_qk(q, kc, s0, gi * S, m)
        m_ref[0, gi] = _finmax(m)

    nba = NT * NG // GA

    def a_body(b, c):
        @pl.when(b % 2 == 0)
        def _():
            a_step(b // 2, 0)

        @pl.when(b % 2 == 1)
        def _():
            a_step(b // 2, 1)
        return c
    jax.lax.fori_loop(0, nba - 1, a_body, 0)
    cp_xb.wait()
    cp_wqkv.wait()

    def matmul_pieces(lhs, rhs, write):
        state = {"acc": None}
        nk, nn = D // 128, D // 512

        def piece(n):
            kt, nh, rb = n % nk, (n // nk) % nn, n // (nk * nn)
            r = jnp.dot(lhs(rb * 128, kt * 128), rhs(kt * 128, nh * 512), preferred_element_type=F32)
            state["acc"] = r if kt == 0 else state["acc"] + r
            if kt == nk - 1:
                write(rb * 128, nh * 512, state["acc"].astype(BF16))
        return piece, (RC // 128) * nn * nk

    def write_k(r0, c0, val):
        for g in range(4):
            kb[c0 // 128 + g, r0:r0 + 128, :] = val[:, g * 128:(g + 1) * 128]

    a_filler, n_pieces = matmul_pieces(
        lambda r, c: xb[r:r + 128, c:c + 128],
        lambda r, c: wqkv[r:r + 128, D + c:D + c + 512], write_k)
    assert n_pieces == GA * nca
    a_step(NT - 1, 1, do_next=False, filler=a_filler)

    cp_woa.wait()
    out_proj(woa, xa, 0, first=0)

    for j in range(nrc):
        x = xb[j * RC:(j + 1) * RC, :]
        if j > 0:
            k = jnp.dot(x, wqkv[:, D:2 * D], preferred_element_type=F32).astype(BF16)
            for g in range(NG):
                kb[g, j * RC:(j + 1) * RC, :] = k[:, g * 128:(g + 1) * 128]
        store_t(proj_t(wqkv[:, 0:D], x, QSCALE), j, qt, 0)
        store_t(proj_t(wqkv[:, 2 * D:3 * D], x), j, vtb, 0)

    def b_load_q(t, g):
        q = qt[t, g * 128:(g + 1) * 128, :]
        z = jnp.zeros((DH, TQ), BF16)
        return jnp.concatenate(
            [jnp.concatenate([q[DH * jj:DH * (jj + 1), :] if jj == j else z for jj in range(4)], axis=0)
             for j in range(4)], axis=1)

    NA = KB // TQ

    def b_blocks(t):
        return range(max(0, NA - 1 - t), NA) if isinstance(t, int) else range(NA)

    def b_qk(t, g, qm, a, s_ref, row0, m):
        k = kb[g, pl.ds(pl.multiple_of((t + a - (NA - 1)) * TQ, TQ), TQ), :]
        s = jnp.dot(k, qm, preferred_element_type=F32)
        if a != 1:
            s = s + jnp.concatenate([bias[a // 2]] * 4, axis=1)
        s_ref[row0 + a * TQ:row0 + (a + 1) * TQ, :] = s
        mc = _colmax(s)
        return mc if m is None else jnp.maximum(m, mc)

    def b_step(t0, par, do_next=True, filler=None):
        s_cur, s_nxt = sbuf[par], sbuf[1 - par]
        n = 0
        hist = [None] * LDEPB
        for ti in range(TB):
            t = t0 + ti
            for g in range(NG):
                u = ti * NG + g
                row0 = u * KB
                if do_next:
                    qm = b_load_q(t + TB, g)
                m_cur = m_ref[par, u]
                m = l = None
                o = [None] * 4
                for a in range(NA):
                    if do_next:
                        m = b_qk(t + TB, g, qm, a, s_nxt, row0, m)
                    if filler is not None:
                        filler(n)
                        n += 1
                    if a not in b_blocks(t):
                        continue
                    s = s_cur[row0 + a * TQ:row0 + (a + 1) * TQ, :].reshape(TQ // 8, 8, 512)
                    mm = m_cur if (not LDEPB or hist[0] is None) else _after(m_cur, hist[0])
                    p = jnp.exp2(s - mm[None])
                    lc = jnp.sum(p, axis=0)
                    l = lc if l is None else l + lc
                    hist = (hist + [l])[1:]
                    p = p.reshape(TQ, 512)
                    for j in range(4):
                        v_t = vtb[t + a - (NA - 1), g * 128 + DH * j:g * 128 + DH * (j + 1), :]
                        oc = jnp.dot(v_t, p[:, j * TQ:(j + 1) * TQ].astype(BF16),
                                     preferred_element_type=F32)
                        o[j] = oc if o[j] is None else o[j] + oc
                if do_next:
                    m_ref[1 - par, u] = _finmax(m)
                l = jnp.sum(l, axis=0, keepdims=True)
                ot[t, g * 128:(g + 1) * 128, :] = jnp.concatenate(
                    [normalise(o[j], l[:, j * TQ:(j + 1) * TQ]).astype(BF16) for j in range(4)],
                    axis=0)

    for ti in range(TB):
        for g in range(NG):
            qm = b_load_q(ti, g)
            m = None
            for a in b_blocks(ti):
                m = b_qk(ti, g, qm, a, s0, (ti * NG + g) * KB, m)
            m_ref[0, ti * NG + g] = _finmax(m)

    nbb = NT // TB
    b_step(0, 0)

    def b_body(b, c):
        @pl.when(b % 2 == 0)
        def _():
            b_step(b * TB, 0)

        @pl.when(b % 2 == 1)
        def _():
            b_step(b * TB, 1)
        return c
    jax.lax.fori_loop(1, nbb - 1, b_body, 0)
    cp_wob.wait()
    oc0 = o_chunk_t(0).T
    nslot = TB * NG * (KB // TQ)

    def write_out0(r0, c0, val):
        xb[r0:r0 + 128, c0:c0 + 512] = val

    o_piece, n_pieces = matmul_pieces(
        lambda r, c: oc0[r:r + 128, c:c + 128],
        lambda r, c: wob[r:r + 128, c:c + 512], write_out0)

    def b_filler(n):
        if n < n_pieces:
            o_piece(n)

    b_step(NT - TB, (nbb - 1) % 2, do_next=False, filler=b_filler)
    for n in range(nslot, n_pieces):
        o_piece(n)

    pieces = [(j, 0, D) for j in range(1, nrc - 1)]
    pieces += [(nrc - 1, c, D // NLAST) for c in range(0, D, D // NLAST)]

    def piece_copy(j, c, n):
        return pltpu.make_async_copy(
            xb.at[pl.ds(j * RC, RC), pl.ds(c, n)],
            out_hbm.at[pl.ds(j * RC, RC), pl.ds(D + c, n)],
            sem_last.at[c // (D // NLAST)] if j == nrc - 1 else sem_out.at[1, j])

    prev, prev_piece = None, (0, 0, D)
    for (j, c, n) in pieces:
        r = jax.lax.dot_general(o_chunk_t(j), wob[:, c:c + n], _TN, preferred_element_type=F32)
        if prev is not None:
            pj, pc, pn = prev_piece
            xb[pj * RC:(pj + 1) * RC, pc:pc + pn] = prev
        piece_copy(*prev_piece).start()
        prev, prev_piece = r.astype(BF16), (j, c, n)
    pj, pc, pn = prev_piece
    xb[pj * RC:(pj + 1) * RC, pc:pc + pn] = prev
    piece_copy(*prev_piece).start()
    for j in range(nrc):
        out_copy(xa, 0, j).wait()
    for piece in [(0, 0, D)] + pieces:
        piece_copy(*piece).wait()


@jax.jit
def pallas_concat_heads__grouped_kv_mqa__sliding_block__prompt_kernel(
    A_x: jax.Array,
    A_wq: jax.Array,
    A_wk: jax.Array,
    A_wv: jax.Array,
    A_wo: jax.Array,
    B_x: jax.Array,
    B_wqkv: jax.Array,
    B_wo: jax.Array,
):
    hbm = pl.BlockSpec(memory_space=pl.ANY)
    scratch = [
        pltpu.VMEM((S, D), BF16),
        pltpu.VMEM((D, D), BF16),
        pltpu.VMEM((2 * DH, D), BF16),
        pltpu.VMEM((D, D), BF16),
        pltpu.VMEM((S, D), BF16),
        pltpu.VMEM((D, 3 * D), BF16),
        pltpu.VMEM((D, D), BF16),
        pltpu.VMEM((NT, D, TQ), BF16),
        pltpu.VMEM((S, DH), BF16),
        pltpu.VMEM((S // RC, DH, RC), BF16),
        pltpu.VMEM((NT, D, TQ), BF16),
        pltpu.VMEM((SROWS, 512), F32),
        pltpu.VMEM((SROWS, 512), F32),
        pltpu.VMEM((2, max(GA, TB * NG), 8, 512), F32),
        pltpu.VMEM((NG, S, 128), BF16),
        pltpu.VMEM((NT, D, TQ), BF16),
        pltpu.VMEM((2, TQ, TQ), F32),
        pltpu.SemaphoreType.DMA((2,)),
        pltpu.SemaphoreType.DMA((NWQ,)),
        pltpu.SemaphoreType.DMA((NX0,)),
        pltpu.SemaphoreType.DMA((S // RC,)),
        pltpu.SemaphoreType.DMA((4,)),
        pltpu.SemaphoreType.DMA((2, S // RC)),
        pltpu.SemaphoreType.DMA((NLAST,)),
    ]
    out = pl.pallas_call(
        _kernel,
        out_shape=jax.ShapeDtypeStruct((S, 2 * D), BF16),
        in_specs=[hbm] * 8,
        out_specs=hbm,
        scratch_shapes=scratch,
        compiler_params=pltpu.CompilerParams(vmem_limit_bytes=100 * 2**20),
    )(A_x.reshape(S, D), A_wq, A_wk.T, A_wv.T, A_wo, B_x.reshape(S, D), B_wqkv, B_wo)
    return out.reshape(1, S, 2 * D)
```

```python
import jax
import jax.numpy as jnp
import jax.experimental.pallas as pl
import jax.experimental.pallas.tpu as pltpu

S = 2048
D = 1024
DH = 32
W = 256
TQ = 128
NT = S // TQ
NG = D // 128
LOG2E = 1.4426950408889634
QSCALE = float(DH ** -0.5) * LOG2E
NEG = -1e9 * LOG2E

KCA = 128
KB = W + TQ
RC = 512
GA = 4
TB = 2
NX0 = 2
KSLICES = (128, 128, 256, 256, 256)
NWQ = len(KSLICES)
NLAST = 4
LAG = 2
SROWS = max(GA * S, TB * NG * KB)

F32 = jnp.float32
BF16 = jnp.bfloat16

_TN_NT = (((0,), (1,)), ((), ()))
_TN = (((0,), (0,)), ((), ()))
_NT = (((1,), (1,)), ((), ()))


def _colmax(s):
    return jnp.max(s.reshape(s.shape[0] // 8, 8, s.shape[1]), axis=0)


def _after(x, dep):
    zero = jax.lax.shift_right_logical(
        jax.lax.shift_right_logical(pltpu.bitcast(dep, jnp.uint32), jnp.uint32(31)), jnp.uint32(1))
    return pltpu.bitcast(pltpu.bitcast(x, jnp.uint32) | zero, x.dtype)


def _finmax(m):
    return jnp.broadcast_to(jnp.max(m, axis=0, keepdims=True), m.shape)


def _kernel(xa_hbm, wq_hbm, wk_hbm, wv_hbm, woa_hbm, xb_hbm, wqkv_hbm, wob_hbm,
            out_hbm,
            xa, wq, wkv, woa, xb, wqkv, wob,
            qt, ka, vta, ot, s0, s1, m_ref, kb, vtb, bias,
            sem_wkv, sem_wq, sem_x0, sem_xa, sem_b, sem_out, sem_last):
    nrc = S // RC
    koff = [sum(KSLICES[:i]) for i in range(len(KSLICES))]

    def rows(hbm, vm, r0, n, sem):
        return pltpu.make_async_copy(hbm.at[pl.ds(r0, n)], vm.at[pl.ds(r0, n)], sem)

    def split(hbm, vm, r0, nr, c0, nc, sems, n):
        return [pltpu.make_async_copy(hbm.at[pl.ds(r0 + k * (nr // n), nr // n), pl.ds(c0, nc)],
                                      vm.at[pl.ds(r0 + k * (nr // n), nr // n), pl.ds(c0, nc)],
                                      sems.at[k]) for k in range(n)]

    cp_wk = pltpu.make_async_copy(wk_hbm, wkv.at[0:DH], sem_wkv.at[0])
    cp_wv = pltpu.make_async_copy(wv_hbm, wkv.at[DH:2 * DH], sem_wkv.at[1])
    pair = [split(xa_hbm, xa, 0, RC, koff[i], KSLICES[i], sem_x0.at[i], NX0 if i == 0 else 1)
            + split(wq_hbm, wq, koff[i], KSLICES[i], 0, D, sem_wq.at[i], 2 * NX0 if i == 0 else 1)
            for i in range(NWQ)]
    cp_xa = [rows(xa_hbm, xa, j * RC, RC, sem_xa.at[j]) for j in range(1, nrc)]
    cp_woa = pltpu.make_async_copy(woa_hbm, woa, sem_b.at[0])
    cp_xb = pltpu.make_async_copy(xb_hbm, xb, sem_b.at[1])
    cp_wqkv = pltpu.make_async_copy(wqkv_hbm, wqkv, sem_b.at[2])
    cp_wob = pltpu.make_async_copy(wob_hbm, wob, sem_b.at[3])
    for cp in (*pair[0], *pair[1], cp_wk, cp_wv):
        cp.start()

    def out_copy(buf, col, j):
        return pltpu.make_async_copy(
            buf.at[pl.ds(j * RC, RC)], out_hbm.at[pl.ds(j * RC, RC), pl.ds(col, D)],
            sem_out.at[col // D, j])

    def o_chunk_t(j):
        return jnp.concatenate([ot[(RC // TQ) * j + i] for i in range(RC // TQ)], axis=1)

    def out_proj(wo, buf, col):
        prev = None
        for j in range(nrc):
            r = jax.lax.dot_general(o_chunk_t(j), wo[...], _TN, preferred_element_type=F32)
            if prev is not None:
                buf[(j - 1) * RC:j * RC, :] = prev
                out_copy(buf, col, j - 1).start()
            prev = r.astype(BF16)
        buf[(nrc - 1) * RC:nrc * RC, :] = prev
        out_copy(buf, col, nrc - 1).start()

    def store_t(r, j, dst):
        for i in range(RC // TQ):
            dst[(RC // TQ) * j + i] = r[:, i * TQ:(i + 1) * TQ]

    def proj_t(w, x, scale=None):
        r = jax.lax.dot_general(w, x, _TN_NT, preferred_element_type=F32)
        if scale is not None:
            r = r * scale
        return r.astype(BF16)

    r = jax.lax.broadcasted_iota(jnp.int32, (TQ, TQ), 0)
    i = jax.lax.broadcasted_iota(jnp.int32, (TQ, TQ), 1)
    bias[0] = jnp.where(r > i, 0.0, NEG).astype(F32)
    bias[1] = jnp.where(r <= i, 0.0, NEG).astype(F32)

    def a_kv(j):
        kv_t = jax.lax.dot_general(wkv[...], xa[j * RC:(j + 1) * RC, :], _NT,
                                   preferred_element_type=F32)
        ka[j * RC:(j + 1) * RC, :] = kv_t[0:DH].T.astype(BF16)
        vta[j] = kv_t[DH:2 * DH].astype(BF16)

    later = [*pair[2:], *[[cp] for cp in cp_xa]]
    r = None
    for i in range(NWQ):
        for cp in pair[i]:
            cp.wait()
        if later:
            for cp in later.pop(0):
                cp.start()
        ks = slice(koff[i], koff[i] + KSLICES[i])
        ri = jnp.dot(xa[0:RC, ks], wq[ks, :], preferred_element_type=F32)
        r = ri if r is None else r + ri
    prev = (r * QSCALE).astype(BF16).T
    while later:
        for cp in later.pop(0):
            cp.start()
    cp_wk.wait()
    cp_wv.wait()
    a_kv(0)
    for j in range(1, nrc):
        cp_xa[j - 1].wait()
        a_kv(j)
        r = proj_t(wq[...], xa[j * RC:(j + 1) * RC, :], QSCALE)
        store_t(prev, j - 1, qt)
        prev = r
    store_t(prev, nrc - 1, qt)
    for cp in (cp_woa, cp_xb, cp_wqkv, cp_wob):
        cp.start()

    sbuf = (s0, s1)
    nca = S // KCA

    def normalise(o, l):
        r = pl.reciprocal(l, approx=True)
        return o * (r * (2.0 - l * r))

    def a_load_q(t, g):
        q = qt[t, g * 128:(g + 1) * 128, :]
        return jnp.concatenate([q[DH * j:DH * (j + 1), :] for j in range(4)], axis=1)

    def a_qk(q, kc, s_ref, row0, m):
        s = jnp.dot(ka[kc * KCA:(kc + 1) * KCA, :], q, preferred_element_type=F32)
        s_ref[row0 + kc * KCA:row0 + (kc + 1) * KCA, :] = s
        mc = _colmax(s)
        return mc if m is None else jnp.maximum(m, mc)

    def a_step(t, par, do_next=True, filler=None):
        s_cur, s_nxt = sbuf[par], sbuf[1 - par]
        for gi in range(GA):
            g = GA * par + gi
            row0 = gi * S
            m_cur = m_ref[par, gi]
            m_nxt = l = o = None
            hist = [None] * LAG
            if do_next:
                q = a_load_q(t + par, GA * (1 - par) + gi)
            for kc in range(nca):
                if do_next:
                    m_nxt = a_qk(q, kc, s_nxt, row0, m_nxt)
                if filler is not None:
                    filler(gi * nca + kc)
                s = s_cur[row0 + kc * KCA:row0 + (kc + 1) * KCA, :].reshape(KCA // 8, 8, 512)
                mm = m_cur if hist[0] is None else _after(m_cur, hist[0])
                p = jnp.exp2(s - mm[None])
                lc = jnp.sum(p, axis=0)
                l = lc if l is None else l + lc
                hist = (hist + [l])[1:]
                k0 = kc * KCA
                v_t = vta[k0 // RC, :, k0 % RC:k0 % RC + KCA]
                oc = jnp.dot(v_t, p.reshape(KCA, 512).astype(BF16), preferred_element_type=F32)
                o = oc if o is None else o + oc
            o = normalise(o, jnp.sum(l, axis=0, keepdims=True))
            ot[t, g * 128:(g + 1) * 128, :] = jnp.concatenate(
                [o[:, j * TQ:(j + 1) * TQ].astype(BF16) for j in range(4)], axis=0)
            if do_next:
                m_ref[1 - par, gi] = _finmax(m_nxt)

    for gi in range(GA):
        q = a_load_q(0, gi)
        m = None
        for kc in range(nca):
            m = a_qk(q, kc, s0, gi * S, m)
        m_ref[0, gi] = _finmax(m)

    nba = NT * NG // GA

    def a_body(b, c):
        @pl.when(b % 2 == 0)
        def _():
            a_step(b // 2, 0)

        @pl.when(b % 2 == 1)
        def _():
            a_step(b // 2, 1)
        return c
    jax.lax.fori_loop(0, nba - 1, a_body, 0)
    cp_xb.wait()
    cp_wqkv.wait()

    def matmul_pieces(lhs, rhs, write):
        state = {"acc": None}
        nk, nn = D // 128, D // 512

        def piece(n):
            kt, nh, rb = n % nk, (n // nk) % nn, n // (nk * nn)
            r = jnp.dot(lhs(rb * 128, kt * 128), rhs(kt * 128, nh * 512), preferred_element_type=F32)
            state["acc"] = r if kt == 0 else state["acc"] + r
            if kt == nk - 1:
                write(rb * 128, nh * 512, state["acc"].astype(BF16))
        return piece, (RC // 128) * nn * nk

    def write_k(r0, c0, val):
        for g in range(4):
            kb[c0 // 128 + g, r0:r0 + 128, :] = val[:, g * 128:(g + 1) * 128]

    a_filler, n_pieces = matmul_pieces(
        lambda r, c: xb[r:r + 128, c:c + 128],
        lambda r, c: wqkv[r:r + 128, D + c:D + c + 512], write_k)
    assert n_pieces == GA * nca
    a_step(NT - 1, 1, do_next=False, filler=a_filler)

    cp_woa.wait()
    out_proj(woa, xa, 0)

    for j in range(nrc):
        x = xb[j * RC:(j + 1) * RC, :]
        if j > 0:
            k = jnp.dot(x, wqkv[:, D:2 * D], preferred_element_type=F32).astype(BF16)
            for g in range(NG):
                kb[g, j * RC:(j + 1) * RC, :] = k[:, g * 128:(g + 1) * 128]
        store_t(proj_t(wqkv[:, 0:D], x, QSCALE), j, qt)
        store_t(proj_t(wqkv[:, 2 * D:3 * D], x), j, vtb)

    def b_load_q(t, g):
        q = qt[t, g * 128:(g + 1) * 128, :]
        z = jnp.zeros((DH, TQ), BF16)
        return jnp.concatenate(
            [jnp.concatenate([q[DH * jj:DH * (jj + 1), :] if jj == j else z for jj in range(4)], axis=0)
             for j in range(4)], axis=1)

    NA = KB // TQ

    def b_blocks(t):
        return range(max(0, NA - 1 - t), NA) if isinstance(t, int) else range(NA)

    def b_qk(t, g, qm, a, s_ref, row0, m):
        k = kb[g, pl.ds(pl.multiple_of((t + a - (NA - 1)) * TQ, TQ), TQ), :]
        s = jnp.dot(k, qm, preferred_element_type=F32)
        if a != 1:
            s = s + jnp.concatenate([bias[a // 2]] * 4, axis=1)
        s_ref[row0 + a * TQ:row0 + (a + 1) * TQ, :] = s
        mc = _colmax(s)
        return mc if m is None else jnp.maximum(m, mc)

    def b_step(t0, par, do_next=True, filler=None):
        s_cur, s_nxt = sbuf[par], sbuf[1 - par]
        n = 0
        hist = [None] * LAG
        for ti in range(TB):
            t = t0 + ti
            for g in range(NG):
                u = ti * NG + g
                row0 = u * KB
                if do_next:
                    qm = b_load_q(t + TB, g)
                m_cur = m_ref[par, u]
                m = l = None
                o = [None] * 4
                for a in range(NA):
                    if do_next:
                        m = b_qk(t + TB, g, qm, a, s_nxt, row0, m)
                    if filler is not None:
                        filler(n)
                        n += 1
                    if a not in b_blocks(t):
                        continue
                    s = s_cur[row0 + a * TQ:row0 + (a + 1) * TQ, :].reshape(TQ // 8, 8, 512)
                    mm = m_cur if hist[0] is None else _after(m_cur, hist[0])
                    p = jnp.exp2(s - mm[None])
                    lc = jnp.sum(p, axis=0)
                    l = lc if l is None else l + lc
                    hist = (hist + [l])[1:]
                    p = p.reshape(TQ, 512)
                    for j in range(4):
                        v_t = vtb[t + a - (NA - 1), g * 128 + DH * j:g * 128 + DH * (j + 1), :]
                        oc = jnp.dot(v_t, p[:, j * TQ:(j + 1) * TQ].astype(BF16),
                                     preferred_element_type=F32)
                        o[j] = oc if o[j] is None else o[j] + oc
                if do_next:
                    m_ref[1 - par, u] = _finmax(m)
                l = jnp.sum(l, axis=0, keepdims=True)
                ot[t, g * 128:(g + 1) * 128, :] = jnp.concatenate(
                    [normalise(o[j], l[:, j * TQ:(j + 1) * TQ]).astype(BF16) for j in range(4)],
                    axis=0)

    for ti in range(TB):
        for g in range(NG):
            qm = b_load_q(ti, g)
            m = None
            for a in b_blocks(ti):
                m = b_qk(ti, g, qm, a, s0, (ti * NG + g) * KB, m)
            m_ref[0, ti * NG + g] = _finmax(m)

    nbb = NT // TB
    b_step(0, 0)

    def b_body(b, c):
        @pl.when(b % 2 == 0)
        def _():
            b_step(b * TB, 0)

        @pl.when(b % 2 == 1)
        def _():
            b_step(b * TB, 1)
        return c
    jax.lax.fori_loop(1, nbb - 1, b_body, 0)
    cp_wob.wait()
    oc0 = o_chunk_t(0).T
    nslot = TB * NG * (KB // TQ)

    def write_out0(r0, c0, val):
        xb[r0:r0 + 128, c0:c0 + 512] = val

    o_piece, n_pieces = matmul_pieces(
        lambda r, c: oc0[r:r + 128, c:c + 128],
        lambda r, c: wob[r:r + 128, c:c + 512], write_out0)

    def b_filler(n):
        if n < n_pieces:
            o_piece(n)

    b_step(NT - TB, (nbb - 1) % 2, do_next=False, filler=b_filler)
    for n in range(nslot, n_pieces):
        o_piece(n)

    pieces = [(j, 0, D) for j in range(1, nrc - 1)]
    pieces += [(nrc - 1, c, D // NLAST) for c in range(0, D, D // NLAST)]

    def piece_copy(j, c, n):
        return pltpu.make_async_copy(
            xb.at[pl.ds(j * RC, RC), pl.ds(c, n)],
            out_hbm.at[pl.ds(j * RC, RC), pl.ds(D + c, n)],
            sem_last.at[c // (D // NLAST)] if j == nrc - 1 else sem_out.at[1, j])

    prev, prev_piece = None, (0, 0, D)
    for (j, c, n) in pieces:
        r = jax.lax.dot_general(o_chunk_t(j), wob[:, c:c + n], _TN, preferred_element_type=F32)
        if prev is not None:
            pj, pc, pn = prev_piece
            xb[pj * RC:(pj + 1) * RC, pc:pc + pn] = prev
        piece_copy(*prev_piece).start()
        prev, prev_piece = r.astype(BF16), (j, c, n)
    pj, pc, pn = prev_piece
    xb[pj * RC:(pj + 1) * RC, pc:pc + pn] = prev
    piece_copy(*prev_piece).start()
    for j in range(nrc):
        out_copy(xa, 0, j).wait()
    for piece in [(0, 0, D)] + pieces:
        piece_copy(*piece).wait()


@jax.jit
def pallas_concat_heads__grouped_kv_mqa__sliding_block__prompt_kernel(
    A_x: jax.Array,
    A_wq: jax.Array,
    A_wk: jax.Array,
    A_wv: jax.Array,
    A_wo: jax.Array,
    B_x: jax.Array,
    B_wqkv: jax.Array,
    B_wo: jax.Array,
):
    hbm = pl.BlockSpec(memory_space=pl.ANY)
    scratch = [
        pltpu.VMEM((S, D), BF16),
        pltpu.VMEM((D, D), BF16),
        pltpu.VMEM((2 * DH, D), BF16),
        pltpu.VMEM((D, D), BF16),
        pltpu.VMEM((S, D), BF16),
        pltpu.VMEM((D, 3 * D), BF16),
        pltpu.VMEM((D, D), BF16),
        pltpu.VMEM((NT, D, TQ), BF16),
        pltpu.VMEM((S, DH), BF16),
        pltpu.VMEM((S // RC, DH, RC), BF16),
        pltpu.VMEM((NT, D, TQ), BF16),
        pltpu.VMEM((SROWS, 512), F32),
        pltpu.VMEM((SROWS, 512), F32),
        pltpu.VMEM((2, max(GA, TB * NG), 8, 512), F32),
        pltpu.VMEM((NG, S, 128), BF16),
        pltpu.VMEM((NT, D, TQ), BF16),
        pltpu.VMEM((2, TQ, TQ), F32),
        pltpu.SemaphoreType.DMA((2,)),
        pltpu.SemaphoreType.DMA((NWQ, 2 * NX0)),
        pltpu.SemaphoreType.DMA((NWQ, NX0)),
        pltpu.SemaphoreType.DMA((S // RC,)),
        pltpu.SemaphoreType.DMA((4,)),
        pltpu.SemaphoreType.DMA((2, S // RC)),
        pltpu.SemaphoreType.DMA((NLAST,)),
    ]
    out = pl.pallas_call(
        _kernel,
        out_shape=jax.ShapeDtypeStruct((S, 2 * D), BF16),
        in_specs=[hbm] * 8,
        out_specs=hbm,
        scratch_shapes=scratch,
        compiler_params=pltpu.CompilerParams(vmem_limit_bytes=100 * 2**20),
    )(A_x.reshape(S, D), A_wq, A_wk.T, A_wv.T, A_wo, B_x.reshape(S, D), B_wqkv, B_wo)
    return out.reshape(1, S, 2 * D)
```
